```python
import os as _os
_os.environ.setdefault("JAX_PLATFORMS", "cpu")
import jax
import jax.numpy as jnp

def _softmax(x, axis=-1):
    return jax.nn.softmax(x, axis=axis)
def _gelu(x):
    return jax.nn.gelu(x, approximate=True)
def _silu(x):
    return jax.nn.silu(x)
def _sigmoid(x):
    return jax.nn.sigmoid(x)
def _layernorm(x, axis=-1, eps=1e-5):
    m = jnp.mean(x, axis=axis, keepdims=True)
    v = jnp.var(x, axis=axis, keepdims=True)
    return (x - m) / jnp.sqrt(v + eps)
def _scatter_add(tgt, idx, src, axis=0):
    return tgt.at[idx].add(src)
def _segment_sum(src, seg, n):
    return jax.ops.segment_sum(src, seg, n)
class _Rng:
    def __init__(self, key):
        self._k = key
    def _next(self):
        self._k, sub = jax.random.split(self._k)
        return sub
    def normal(self, shape):
        return jax.random.normal(self._next(), shape, dtype=jnp.bfloat16)
    def randint(self, lo, hi, shape):
        return jax.random.randint(self._next(), shape, lo, hi, dtype=jnp.int32)
    def uniform(self, shape, lo=0.0, hi=1.0):
        return jax.random.uniform(self._next(), shape, jnp.bfloat16, lo, hi)
    def permutation(self, n):
        return jax.random.permutation(self._next(), n)


kernel_name = 'concat_heads__sliding_block_cached__sliding_block_cached__decode'

def setup_inputs():
    _rng = _Rng(jax.random.key(int.from_bytes(__import__("os").urandom(4), "little")))
    _w = (lambda a: (lambda t: t.astype(jnp.bfloat16) if jnp.issubdtype(t.dtype, jnp.floating) else t)(jnp.asarray(a)))
    def _A_setup():
        B, Sq, D = 1, 1, 640
        Hq, Hkv, Sk, Dh = 32, 32, 4096, 192
        assert Hq % Hkv == 0, (Hq, Hkv)
        return {
            "x": _w((lambda *s: _rng.normal(s) * 0.8)(B, Sq, D)),
            "k_cache": _w((lambda *s: _rng.normal(s) * 0.8)(B, Hkv, Sk, Dh)),
            "v_cache": _w((lambda *s: _rng.normal(s) * 0.05)(B, Hkv, Sk, Dh)),
            "wq": _w((lambda *s: _rng.normal(s) * 0.8)(D, Hq * Dh) * (D ** -0.5)),
            "wo": _w((lambda *s: _rng.normal(s) * 0.05)(Hq * Dh, D) * ((Hq * Dh) ** -0.5)),
        }
    _A_in = _A_setup()

    def _B_setup():
        B, Sq, D = 1, 1, 640
        Hq, Hkv, Sk, Dh = 32, 32, 4096, 192
        assert Hq % Hkv == 0, (Hq, Hkv)
        return {
            "x": _w((lambda *s: _rng.normal(s) * 0.8)(B, Sq, D)),
            "k_cache": _w((lambda *s: _rng.normal(s) * 0.8)(B, Hkv, Sk, Dh)),
            "v_cache": _w((lambda *s: _rng.normal(s) * 0.05)(B, Hkv, Sk, Dh)),
            "wq": _w((lambda *s: _rng.normal(s) * 0.8)(D, Hq * Dh) * (D ** -0.5)),
            "wo": _w((lambda *s: _rng.normal(s) * 0.05)(Hq * Dh, D) * ((Hq * Dh) ** -0.5)),
        }
    _B_in = _B_setup()

    return {
        "A_x": _A_in["x"],
        "A_k_cache": _A_in["k_cache"],
        "A_v_cache": _A_in["v_cache"],
        "A_wq": _A_in["wq"],
        "A_wo": _A_in["wo"],
        "B_x": _B_in["x"],
        "B_k_cache": _B_in["k_cache"],
        "B_v_cache": _B_in["v_cache"],
        "B_wq": _B_in["wq"],
        "B_wo": _B_in["wo"],
    }

def reference(A_x, A_k_cache, A_v_cache, A_wq, A_wo, B_x, B_k_cache, B_v_cache, B_wq, B_wo):
    def _A_ref(x, k_cache, v_cache, wq, wo):
        B, Sq, D = x.shape
        Hq, Dh = 32, 192
        Hkv, Sk = k_cache.shape[1], k_cache.shape[2]
        W = min(4096, max(256, Sk // 4))
        rep = Hq // Hkv
        q = (lambda x, *d: x.transpose(*d))((x @ wq).reshape(B, Sq, Hq, Dh), 0, 2, 1, 3)
        k = jnp.repeat(k_cache[:, :, Sk - W:, :], rep, axis=1)
        v = jnp.repeat(v_cache[:, :, Sk - W:, :], rep, axis=1)
        scores = jnp.einsum("bhqd,bhkd->bhqk", q, k) * (Dh ** -0.5)
        p = _softmax(scores, axis=-1)
        o = jnp.einsum("bhqk,bhkd->bhqd", p, v)
        return (lambda x, *d: x.transpose(*d))(o, 0, 2, 1, 3).reshape(B, Sq, Hq * Dh) @ wo

    def _B_ref(x, k_cache, v_cache, wq, wo):
        B, Sq, D = x.shape
        Hq, Dh = 32, 192
        Hkv, Sk = k_cache.shape[1], k_cache.shape[2]
        W = min(4096, max(256, Sk // 4))
        rep = Hq // Hkv
        q = (lambda x, *d: x.transpose(*d))((x @ wq).reshape(B, Sq, Hq, Dh), 0, 2, 1, 3)
        k = jnp.repeat(k_cache[:, :, Sk - W:, :], rep, axis=1)
        v = jnp.repeat(v_cache[:, :, Sk - W:, :], rep, axis=1)
        scores = jnp.einsum("bhqd,bhkd->bhqk", q, k) * (Dh ** -0.5)
        p = _softmax(scores, axis=-1)
        o = jnp.einsum("bhqk,bhkd->bhqd", p, v)
        return (lambda x, *d: x.transpose(*d))(o, 0, 2, 1, 3).reshape(B, Sq, Hq * Dh) @ wo

    a = _A_ref(A_x, A_k_cache, A_v_cache, A_wq, A_wo)
    b = _B_ref(B_x, B_k_cache, B_v_cache, B_wq, B_wo)
    return jnp.concatenate([a, b], axis=-1)
```

```python
import jax
import jax.numpy as jnp
from jax import lax
import jax.experimental.pallas as pl
import jax.experimental.pallas.tpu as pltpu

H, DH, SK, W, D = 32, 192, 4096, 1024, 640
NI = 32
ROT = 25
bf16, f32 = jnp.bfloat16, jnp.float32


def _divmod(i, c):
    if c & (c - 1) == 0:
        return i >> (c.bit_length() - 1), i & (c - 1)
    q = lax.div(i, jnp.int32(c))
    return q, i - q * c


def _kernel(ax, ak, av, awq, awo, bx, bk, bv, bwq, bwo, o_ref,
            qb, kb, vb, ob, xb, xe, qacc, qs, sacc, pb, linv, o2d, oe, oacc, sems, osems):
    sub = lax.broadcasted_iota(jnp.int32, (8, 128), 0)
    lane = lax.broadcasted_iota(jnp.int32, (8, 128), 1)

    def kv_pair(src, dst, half, sem):
        def issue(i, u):
            for q in (1, 0):
                p = i * 4 + u
                if q == 0:
                    p = (p - ROT) & (NI * 4 - 1)
                j, c = _divmod(p, 16)
                gs = pl.ds(half * 48 + c * 3 + q, 1 + q)
                rs = pl.ds(pl.multiple_of(j * 8, 8), 8)
                pltpu.make_async_copy(src.at[gs, rs, pl.ds(SK - W, W)], dst.at[gs, rs], sem).start(priority=q)
        return 4, issue

    def w_pair(src, dst, rows, sem_of, rot):
        def issue(i, u):
            for q in (1, 0):
                j, c = i, u
                if q == 0 and rot:
                    dj, c = divmod(u - rot, 5)
                    j = (i + dj) & (NI - 1)
                gs = pl.ds(c * 3 + q, 1 + q)
                rs = pl.ds(pl.multiple_of(j * rows, rows), rows)
                pltpu.make_async_copy(src.at[gs, rs], dst.at[gs, rs], sem_of(j)).start(priority=q)
        return 5, issue

    def wait(dst, sem):
        pltpu.make_async_copy(dst, dst, sem).wait()

    def row(ref, a, b):
        return jnp.broadcast_to(ref[a, pl.ds(b, 1), :], (8, 128))

    def headmask(c):
        rel = lane + c * 128 - sub * DH
        return (rel >= 0) & (rel < DH)

    def expand(x, rep):
        k = lax.broadcasted_iota(jnp.int32, (128, 128), 0)
        n = lax.broadcasted_iota(jnp.int32, (128, 128), 1)
        outs = []
        for m in range(rep):
            t = (n >> 3) + 16 * m - (k >> 3) * rep
            e = jnp.where((t >= 0) & (t < rep) & ((n & 7) == (k & 7)), 1.0, 0.0).astype(bf16)
            outs.append(jnp.dot(x, e, preferred_element_type=f32))
        return outs

    def tilemask(m, rep):
        t = (lane >> 3) + 16 * m
        q = (t * (65536 // rep + 1)) >> 16
        return t - q * rep == sub

    def xprep():
        rows = [xb[b, 0, :, pl.ds(128 * k, 128)].astype(f32) for b in range(2) for k in range(5)]
        x = jnp.concatenate(rows + [jnp.zeros((6, 128), f32)], axis=0).astype(bf16)
        for m, e in enumerate(expand(x, 6)):
            xe[m] = e

    def qproj(b):
        def step(i):
            k, m = _divmod(i, 6)
            l = jnp.where(tilemask(m, 6), row(xe, m, b * 5 + k), 0.0).astype(bf16)
            w = qb[b, i >> 1, pl.ds(pl.multiple_of((i & 1) * 128, 128), 128), :]
            qacc[b] += jnp.dot(l, w, preferred_element_type=f32)
        return step

    def qk(b, half):
        def step(i):
            i = i + 24 * half
            g, c = _divmod(i, 12)
            l = jnp.where(headmask(c), row(qs.at[b], i & 7, i >> 3), 0.0).astype(bf16)
            sacc[b, g] += jnp.dot(l, kb[b, pl.ds(2 * i, 2)].reshape(128, W), preferred_element_type=f32)
        return step

    def softmax(b, half):
        for g in (2 * half, 2 * half + 1):
            s = sacc[b, g] * (DH ** -0.5)
            e = jnp.exp(s - jnp.max(s, axis=-1, keepdims=True))
            pb[b, g] = e
            linv[b, g] = jnp.broadcast_to(1.0 / jnp.sum(e, axis=-1, keepdims=True), (8, 128))

    def pv(b, half):
        def step(i):
            i = i + 24 * half
            g, c = _divmod(i, 12)
            o = lax.dot_general(pb[b, g].astype(bf16), vb[b, pl.ds(2 * i, 2)].reshape(128, W),
                                (((1,), (1,)), ((), ())), preferred_element_type=f32)
            o2d[b, pl.ds(i, 1), :] = jnp.sum(jnp.where(headmask(c), o * linv[b, g], 0.0), axis=0, keepdims=True)
        return step

    def oproj(b, jj):
        s = oacc[b]
        for g in range(15):
            i, m = _divmod(g * 16 + jj, 5)
            l = jnp.where(tilemask(m, 5), row(oe, m, b * 48 + i), 0.0).astype(bf16)
            w = ob[b, g, pl.ds(pl.multiple_of(jj * 128, 128), 128), :]
            s = s + jnp.dot(l, w, preferred_element_type=f32)
        oacc[b] = s

    def loop(lo, hi, pair, step=None, off=0):
        n, issue = pair

        def body(i, carry):
            for u in range(n):
                issue(i, u)
                if step is not None and u == n // 2 - 1:
                    step(i - off)
            return carry
        if hi > lo:
            lax.fori_loop(lo, hi, body, 0)

    def block(pair, pre, landed, step, st):
        loop(0, 1, pair)
        if pre is not None:
            pre()
        loop(1, st, pair)
        wait(*landed)
        loop(st, st + 24, pair, step, st)
        loop(st + 24, NI, pair)

    def kvp(src, buf, b, half, s):
        return kv_pair(src, buf.at[b], half, sems.at[s])

    def kvw(buf, b, half, s):
        return buf.at[b, pl.ds(48 * half, 48)], sems.at[s]

    xc = [pltpu.make_async_copy(x, xb.at[i], sems.at[11]) for i, x in enumerate((ax, bx))]
    p = w_pair(awq, qb.at[0], 8, lambda j: sems.at[0], ROT)
    loop(0, 4, p)
    for c in xc:
        c.start()
    qacc[...] = jnp.zeros(qacc.shape, f32)
    sacc[...] = jnp.zeros(sacc.shape, f32)
    oacc[...] = jnp.zeros(oacc.shape, f32)
    loop(4, 16, p)
    for c in xc:
        c.wait()
    xprep()
    loop(16, NI, p)

    p = w_pair(bwq, qb.at[1], 8, lambda j: sems.at[1], ROT)
    loop(0, 6, p)
    wait(qb.at[0], sems.at[0])
    loop(6, NI, p, qproj(0), 6)
    p = kvp(ak, kb, 0, 0, 2)
    loop(0, 4, p, qproj(0), -26)
    loop(4, 8, p)
    wait(qb.at[1], sems.at[1])
    loop(8, NI, p, qproj(1), 8)
    p = kvp(ak, kb, 0, 1, 3)
    loop(0, 6, p, qproj(1), -24)
    for b in range(2):
        for n in range(8):
            qs[b, n] = qacc[b, :, pl.ds(128 * n, 128)]
    loop(6, 8, p)
    wait(*kvw(kb, 0, 0, 2))
    loop(8, NI, p, qk(0, 0), 8)
    block(kvp(bk, kb, 1, 0, 4), lambda: softmax(0, 0), kvw(kb, 0, 1, 3), qk(0, 1), 8)
    block(kvp(bk, kb, 1, 1, 5), lambda: softmax(0, 1), kvw(kb, 1, 0, 4), qk(1, 0), 8)
    block(kvp(av, vb, 0, 0, 6), lambda: softmax(1, 0), kvw(kb, 1, 1, 5), qk(1, 1), 8)
    block(kvp(av, vb, 0, 1, 7), lambda: softmax(1, 1), kvw(vb, 0, 0, 6), pv(0, 0), 8)
    block(kvp(bv, vb, 1, 0, 8), None, kvw(vb, 0, 1, 7), pv(0, 1), 8)
    block(kvp(bv, vb, 1, 1, 9), None, kvw(vb, 1, 0, 8), pv(1, 0), 8)
    block(w_pair(awo, ob.at[0], 64, lambda j: sems.at[10], ROT), None, kvw(vb, 1, 1, 9), pv(1, 1), 6)

    p = w_pair(bwo, ob.at[1], 64, lambda j: osems.at[j >> 1], 0)
    loop(0, 1, p)
    for m, e in enumerate(expand(o2d[...].reshape(96, 128).astype(bf16), 5)):
        oe[m] = e
    loop(1, 6, p)
    wait(ob.at[0], sems.at[10])
    loop(6, 22, p, lambda jj: oproj(0, jj), 6)

    def ostep(jj):
        wait(ob.at[1, :, pl.ds(pl.multiple_of(jj * 128, 128), 128)], osems.at[jj])
        oproj(1, jj)

    loop(22, NI, p, ostep, 22)
    for c in range(5):
        o_ref[0, :, pl.ds(128 * c, 128)] = oacc[0, pl.ds(c, 1), :].astype(bf16)

    def tail(jj, carry):
        ostep(jj)
        return carry
    lax.fori_loop(10, 16, tail, 0)
    for c in range(5):
        o_ref[0, :, pl.ds(D + 128 * c, 128)] = oacc[1, pl.ds(c, 1), :].astype(bf16)


@jax.jit
def pallas_concat_heads__sliding_block_cached__sliding_block_cached__decode_kernel(
    A_x: jax.Array,
    A_k_cache: jax.Array,
    A_v_cache: jax.Array,
    A_wq: jax.Array,
    A_wo: jax.Array,
    B_x: jax.Array,
    B_k_cache: jax.Array,
    B_v_cache: jax.Array,
    B_wq: jax.Array,
    B_wo: jax.Array,
):
    def kv_view(t):
        return jnp.swapaxes(t, 2, 3).reshape(96, 64, SK)

    def wq_view(t):
        return t.reshape(80, 8, 6, 1024).transpose(0, 2, 1, 3).reshape(15, 256, 1024)

    def wo_view(t):
        return t.reshape(768, 8, 5, 128).transpose(0, 2, 1, 3).reshape(15, 2048, 128)

    return pl.pallas_call(
        _kernel,
        in_specs=[pl.BlockSpec(memory_space=pltpu.HBM)] * 10,
        out_specs=pl.BlockSpec(memory_space=pltpu.VMEM),
        out_shape=jax.ShapeDtypeStruct((1, 1, 2 * D), bf16),
        scratch_shapes=[
            pltpu.VMEM((2, 15, 256, 1024), bf16),
            pltpu.VMEM((2, 96, 64, W), bf16),
            pltpu.VMEM((2, 96, 64, W), bf16),
            pltpu.VMEM((2, 15, 2048, 128), bf16),
            pltpu.VMEM((2, 1, 1, D), bf16),
            pltpu.VMEM((6, 16, 128), f32),
            pltpu.VMEM((2, 8, 1024), f32),
            pltpu.VMEM((2, 8, 8, 128), f32),
            pltpu.VMEM((2, 4, 8, W), f32),
            pltpu.VMEM((2, 4, 8, W), f32),
            pltpu.VMEM((2, 4, 8, 128), f32),
            pltpu.VMEM((2, 48, 128), f32),
            pltpu.VMEM((5, 96, 128), f32),
            pltpu.VMEM((2, 8, 128), f32),
            pltpu.SemaphoreType.DMA((12,)),
            pltpu.SemaphoreType.DMA((16,)),
        ],
        compiler_params=pltpu.CompilerParams(
            vmem_limit_bytes=100 * 2**20,
            disable_bounds_checks=True,
            disable_semaphore_checks=True,
        ),
    )(A_x, kv_view(A_k_cache), kv_view(A_v_cache), wq_view(A_wq), wo_view(A_wo),
      B_x, kv_view(B_k_cache), kv_view(B_v_cache), wq_view(B_wq), wo_view(B_wo))
```

```python
import jax
import jax.numpy as jnp
from jax import lax
import jax.experimental.pallas as pl
import jax.experimental.pallas.tpu as pltpu

H, DH, SK, D = 32, 192, 4096, 640
W = min(4096, max(256, SK // 4))
LEAD = 24
bf16, f32 = jnp.bfloat16, jnp.float32


def _divmod(i, c):
    if isinstance(i, int):
        return divmod(i, c)
    q = (i * (65536 // c + 1)) >> 16
    return q, i - q * c


def _rows(i, n, offset=0, size=None):
    size = size or n
    start = i * n + offset
    return pl.ds(start if isinstance(start, int) else pl.multiple_of(start, size), size)


def _kernel(ax, ak, av, awq, awo, bx, bk, bv, bwq, bwo, out_hbm,
            wq_buf, k_buf, v_buf, wo_buf, x_buf, x_rep, q_acc, p_buf, o_col, out_acc, out_buf, pace_buf,
            sems, sweep_sems):
    sub = lax.broadcasted_iota(jnp.int32, (8, 128), 0)
    lane = lax.broadcasted_iota(jnp.int32, (8, 128), 1)

    def groups(first, n, prio):
        return pl.ds(first + 1, n) if prio else pl.ds(first, 1)

    def kv_stream(src, dst, sem):
        def copy(i, u, prio):
            g = groups((i & 3) * 24 + (u // 2) * 6, 5, prio)
            r, c = _rows(i >> 2, 8), (u % 2) * (W // 2)
            return pltpu.make_async_copy(
                src.at[g, r, pl.ds(SK - W + c, W // 2)], dst.at[g, r, pl.ds(c, W // 2)], sem)
        return 8, copy

    def wq_stream(src, dst, sem):
        def copy(i, u, prio):
            idx = (groups((u % 3) * 5, 4, prio), _rows(i, 8), pl.ds((u // 3) * 512, 512))
            return pltpu.make_async_copy(src.at[idx], dst.at[idx], sem)
        return 6, copy

    def wo_stream(src, dst, sem_of):
        def copy(i, u, prio):
            idx = (groups((u % 3) * 5, 4, prio), _rows(i, 64, (u // 3) * 32, 32))
            return pltpu.make_async_copy(src.at[idx], dst.at[idx], sem_of(i, u))
        return 6, copy

    def pace(i, u, prio):
        src = (ax, bx)[u % 2].at[0, :, pl.ds(128 * (u // 2 % 5), 128)]
        return pltpu.make_async_copy(src, pace_buf.at[u], sems.at[8])

    def wait(dst, sem):
        pltpu.make_async_copy(dst, dst, sem).wait()

    def handover(prev, nxt):
        for p in range(LEAD):
            nxt[1](*divmod(p, nxt[0]), 1).start(priority=1)
            if prev is not None:
                prev[1](*divmod(32 * prev[0] - LEAD + p, prev[0]), 0).start(priority=0)

    def run(stream, lo, hi, step=None):
        n, copy = stream

        def body(i, carry):
            for u in range(n):
                copy(i + LEAD // n, u, 1).start(priority=1)
                copy(i, u, 0).start(priority=0)
            if step is not None:
                step(i - lo)
            return carry
        lax.fori_loop(lo, hi, body, 0)

    def row(ref, a, b):
        return jnp.broadcast_to(ref[a, pl.ds(b, 1), :], (8, 128))

    def repeat_x():
        k = lax.broadcasted_iota(jnp.int32, (128, 128), 0)
        n = lax.broadcasted_iota(jnp.int32, (128, 128), 1)
        xs = [x_buf[b, 0, :, pl.ds(128 * i, 128)].astype(f32) for b in range(2) for i in range(5)]
        x = jnp.concatenate(xs + [jnp.zeros((6, 128), f32)], axis=0).astype(bf16)
        for m in range(6):
            t = (n >> 3) + 16 * m - (k >> 3) * 6
            pick = jnp.where((t >= 0) & (t < 6) & ((n & 7) == (k & 7)), 1.0, 0.0).astype(bf16)
            x_rep[m] = jnp.dot(x, pick, preferred_element_type=f32)

    def q_proj(b):
        def step(g):
            lhs = []
            for h in range(2):
                k, m = _divmod(2 * g + h, 6)
                mine = _divmod((lane >> 3) + 16 * m, 6)[1] == sub
                lhs.append(jnp.where(mine, row(x_rep, m, 5 * b + k), 0.0))
            lhs = jnp.concatenate(lhs, axis=1).astype(bf16)
            q = jnp.dot(lhs, wq_buf[b, g], preferred_element_type=f32)
            for n in range(8):
                q_acc[b, n] += q[:, 128 * n:128 * (n + 1)]
        return step

    def attention_probs(b):
        def step(i):
            lhs = []
            for c in range(3):
                t = 3 * i + c
                d = lane + 128 * c - sub * DH
                lhs.append(jnp.where((d >= 0) & (d < DH), row(q_acc.at[b], t & 7, t >> 3), 0.0))
            lhs = jnp.concatenate(lhs, axis=1).astype(bf16)
            kt = k_buf[b, pl.ds(6 * i, 6)].reshape(2 * DH, W)
            s = jnp.dot(lhs, kt, preferred_element_type=f32) * (DH ** -0.5)
            e = jnp.exp(s - jnp.max(s, axis=-1, keepdims=True))
            p_buf[b, i] = e / jnp.sum(e, axis=-1, keepdims=True)
        return step

    def weighted_values(b):
        def step(i):
            for g in range(6):
                p = p_buf[b, i, pl.ds(g // 3, 1), :]
                o = jnp.sum(v_buf[b, 6 * i + g].astype(f32) * p, axis=-1, keepdims=True)
                o_col[b, pl.ds((6 * i + g) * 8, 8)] = jnp.broadcast_to(o, (64, 128)).reshape(8, 8, 128)
        return step

    def out_proj(b, j, gs, acc, tiles=range(8)):
        a, r = _divmod(8 * j, 5)
        base = [a + _divmod(r + k, 5)[0] for k in range(5)]
        for g in gs:
            w = wo_buf[b, g, _rows(j, 64, 8 * tiles[0], 8 * len(tiles)), :].astype(f32)
            for n, i in enumerate(tiles):
                a2, k = divmod(256 * g + i, 5)
                acc[k] = acc[k] + w[8 * n:8 * n + 8] * o_col[b, base[k] + a2]
        return acc

    def out_sweeps(b, lo, n):
        def body(j, carry):
            j = lo + j
            if b == 1:
                wait(wo_buf.at[1, :, _rows(j, 64)], sweep_sems.at[j])
            slot = [_divmod(k + 3 * j, 5)[1] for k in range(5)]
            acc = out_proj(b, j, range(15), [out_acc[b, s] for s in slot])
            for s, v in zip(slot, acc):
                out_acc[b, s] = v
            return carry
        lax.fori_loop(0, n, body, 0)

    def out_copy(b):
        half = (slice(None), slice(None), pl.ds(b * D, D))
        return pltpu.make_async_copy(out_buf.at[half], out_hbm.at[half], sems.at[9 + b])

    def write_out(b, acc):
        for c in range(5):
            out_buf[0, :, pl.ds(b * D + 128 * c, 128)] = jnp.sum(acc[c], axis=0, keepdims=True).astype(bf16)
        out_copy(b).start()

    def wo_b_sem(j, u):
        return sweep_sems.at[j + (u - 2) * ((j + 1) >> 5) if u >= 3 else j]

    bufs = [wq_buf.at[0], wq_buf.at[1], k_buf.at[0], k_buf.at[1], v_buf.at[0], v_buf.at[1], wo_buf.at[0]]
    streams = [
        wq_stream(awq, bufs[0], sems.at[0]), wq_stream(bwq, bufs[1], sems.at[1]),
        kv_stream(ak, bufs[2], sems.at[2]), kv_stream(bk, bufs[3], sems.at[3]),
        kv_stream(av, bufs[4], sems.at[4]), kv_stream(bv, bufs[5], sems.at[5]),
        wo_stream(awo, bufs[6], lambda j, u: sems.at[6]), wo_stream(bwo, wo_buf.at[1], wo_b_sem),
    ]
    jobs = [(15, q_proj(0)), (15, q_proj(1)), (16, attention_probs(0)), (16, attention_probs(1)),
            (16, weighted_values(0)), (16, weighted_values(1)), (8, lambda i: out_sweeps(0, 4 * i, 4))]

    handover(None, streams[0])
    x_copies = [pltpu.make_async_copy(x, x_buf.at[b], sems.at[7]) for b, x in enumerate((ax, bx))]
    for c in x_copies:
        c.start()
    run(streams[0], 0, 14)
    q_acc[...] = jnp.zeros(q_acc.shape, f32)
    out_acc[...] = jnp.zeros(out_acc.shape, f32)
    for c in x_copies:
        c.wait()
    repeat_x()
    run(streams[0], 14, 28)

    for s, (steps, step) in enumerate(jobs):
        stream = streams[s + 1]
        end = 32 - LEAD // stream[0]
        start = 8 if s == 6 else end - steps
        handover(streams[s], stream)
        run(stream, 0, start)
        wait(bufs[s], sems.at[s])
        run(stream, start, start + steps, step)

    write_out(0, [out_acc[0, c] for c in range(5)])
    run(streams[7], 16, 19)
    run(streams[7], 19, 28, lambda i: out_sweeps(1, 2 * i, 2))
    handover(streams[7], (LEAD, pace))

    out_sweeps(1, 18, 13)
    acc = [out_acc[1, (k + 3 * 31) % 5] for k in range(5)]
    wait(wo_buf.at[1, :, _rows(31, 64, 0, 32)], sweep_sems.at[31])
    acc = out_proj(1, 31, range(15), acc, range(4))
    for u in range(3):
        wait(wo_buf.at[1, pl.ds(5 * u, 5), _rows(31, 64, 32, 32)], sweep_sems.at[32 + u])
        acc = out_proj(1, 31, range(5 * u, 5 * u + 5), acc, range(4, 8))
    write_out(1, [acc[(c - 3 * 31) % 5] for c in range(5)])
    out_copy(0).wait()
    wait(pace_buf, sems.at[8])
    out_copy(1).wait()


@jax.jit
def pallas_concat_heads__sliding_block_cached__sliding_block_cached__decode_kernel(
    A_x: jax.Array,
    A_k_cache: jax.Array,
    A_v_cache: jax.Array,
    A_wq: jax.Array,
    A_wo: jax.Array,
    B_x: jax.Array,
    B_k_cache: jax.Array,
    B_v_cache: jax.Array,
    B_wq: jax.Array,
    B_wo: jax.Array,
):
    def kv_view(t):
        return jnp.swapaxes(t, 2, 3).reshape(96, 64, SK)

    def wq_view(t):
        return t.reshape(80, 8, 6, 1024).transpose(0, 2, 1, 3).reshape(15, 256, 1024)

    def wo_view(t):
        return t.reshape(768, 8, 5, 128).transpose(0, 2, 1, 3).reshape(15, 2048, 128)

    hbm = pl.BlockSpec(memory_space=pltpu.HBM)
    return pl.pallas_call(
        _kernel,
        in_specs=[hbm] * 10,
        out_specs=hbm,
        out_shape=jax.ShapeDtypeStruct((1, 1, 2 * D), bf16),
        scratch_shapes=[
            pltpu.VMEM((2, 15, 256, 1024), bf16),
            pltpu.VMEM((2, 96, 64, W), bf16),
            pltpu.VMEM((2, 96, 64, W), bf16),
            pltpu.VMEM((2, 15, 2048, 128), bf16),
            pltpu.VMEM((2, 1, 1, D), bf16),
            pltpu.VMEM((6, 16, 128), f32),
            pltpu.VMEM((2, 8, 8, 128), f32),
            pltpu.VMEM((2, H // 2, 8, W), f32),
            pltpu.VMEM((2, 768, 8, 128), f32),
            pltpu.VMEM((2, 5, 8, 128), f32),
            pltpu.VMEM((1, 1, 2 * D), bf16),
            pltpu.VMEM((LEAD, 1, 128), bf16),
            pltpu.SemaphoreType.DMA((11,)),
            pltpu.SemaphoreType.DMA((35,)),
        ],
        compiler_params=pltpu.CompilerParams(
            vmem_limit_bytes=100 * 2**20,
            disable_bounds_checks=True,
            disable_semaphore_checks=True,
        ),
    )(A_x, kv_view(A_k_cache), kv_view(A_v_cache), wq_view(A_wq), wo_view(A_wo),
      B_x, kv_view(B_k_cache), kv_view(B_v_cache), wq_view(B_wq), wo_view(B_wo))
```

```python
import jax
import jax.numpy as jnp
from jax import lax
import jax.experimental.pallas as pl
import jax.experimental.pallas.tpu as pltpu

H, DH, SK, D = 32, 192, 4096, 640
W = min(4096, max(256, SK // 4))
LEAD = 24
bf16, f32 = jnp.bfloat16, jnp.float32


def _divmod(i, c):
    if isinstance(i, int):
        return divmod(i, c)
    q = (i * (65536 // c + 1)) >> 16
    return q, i - q * c


def _rows(i, n, offset=0, size=None):
    size = size or n
    start = i * n + offset
    return pl.ds(start if isinstance(start, int) else pl.multiple_of(start, size), size)


def _kernel(ax, ak, av, awq, awo, bx, bk, bv, bwq, bwo, out_hbm,
            wq_buf, k_buf, v_buf, wo_buf, x_buf, x_rep, q_acc, p_buf, o_col, out_acc, out_buf,
            sems, sweep_sems):
    sub = lax.broadcasted_iota(jnp.int32, (8, 128), 0)
    lane = lax.broadcasted_iota(jnp.int32, (8, 128), 1)

    def groups(first, n, prio):
        return pl.ds(first + 1, n) if prio else pl.ds(first, 1)

    def kv_stream(src, dst, sem):
        def copy(i, u, prio):
            g = groups((i & 3) * 24 + (u // 2) * 6, 5, prio)
            r, c = _rows(i >> 2, 8), (u % 2) * (W // 2)
            return pltpu.make_async_copy(
                src.at[g, r, pl.ds(SK - W + c, W // 2)], dst.at[g, r, pl.ds(c, W // 2)], sem)
        return 8, copy

    def wq_stream(src, dst, sem):
        def copy(i, u, prio):
            idx = (groups((u % 3) * 5, 4, prio), _rows(i, 8), pl.ds((u // 3) * 512, 512))
            return pltpu.make_async_copy(src.at[idx], dst.at[idx], sem)
        return 6, copy

    def wo_stream(src, dst, sem_of, num_groups=15):
        def copy(i, u, prio):
            first = (u % 3) * 5
            idx = (groups(first, min(4, num_groups - first - 1), prio), _rows(i, 64, (u // 3) * 32, 32))
            return pltpu.make_async_copy(src.at[idx], dst.at[idx], sem_of(i))
        return 6, copy

    def wait(dst, sem):
        pltpu.make_async_copy(dst, dst, sem).wait()

    def handover(prev, nxt):
        for p in range(LEAD):
            nxt[1](*divmod(p, nxt[0]), 1).start(priority=0 if prev is None and p == 2 else 1)
            if prev is not None:
                prev[1](*divmod(32 * prev[0] - LEAD + p, prev[0]), 0).start(priority=0)

    def run(stream, lo, hi, step=None):
        n, copy = stream

        def body(i, carry):
            for u in range(n):
                copy(i + LEAD // n, u, 1).start(priority=1)
                copy(i, u, 0).start(priority=0)
            if step is not None:
                step(i - lo)
            return carry
        lax.fori_loop(lo, hi, body, 0)

    def row(ref, a, b):
        return jnp.broadcast_to(ref[a, pl.ds(b, 1), :], (8, 128))

    def repeat_x():
        k = lax.broadcasted_iota(jnp.int32, (128, 128), 0)
        n = lax.broadcasted_iota(jnp.int32, (128, 128), 1)
        xs = [x_buf[b, 0, :, pl.ds(128 * i, 128)].astype(f32) for b in range(2) for i in range(5)]
        x = jnp.concatenate(xs + [jnp.zeros((6, 128), f32)], axis=0).astype(bf16)
        for m in range(6):
            t = (n >> 3) + 16 * m - (k >> 3) * 6
            pick = jnp.where((t >= 0) & (t < 6) & ((n & 7) == (k & 7)), 1.0, 0.0).astype(bf16)
            x_rep[m] = jnp.dot(x, pick, preferred_element_type=f32)

    def q_proj(b):
        def step(g):
            lhs = []
            for h in range(2):
                k, m = _divmod(2 * g + h, 6)
                mine = _divmod((lane >> 3) + 16 * m, 6)[1] == sub
                lhs.append(jnp.where(mine, row(x_rep, m, 5 * b + k), 0.0))
            lhs = jnp.concatenate(lhs, axis=1).astype(bf16)
            q = jnp.dot(lhs, wq_buf[b, g], preferred_element_type=f32)
            for n in range(8):
                q_acc[b, n] += q[:, 128 * n:128 * (n + 1)]
        return step

    def attention_probs(b):
        def step(i):
            lhs = []
            for c in range(3):
                t = 3 * i + c
                d = lane + 128 * c - sub * DH
                lhs.append(jnp.where((d >= 0) & (d < DH), row(q_acc.at[b], t & 7, t >> 3), 0.0))
            lhs = jnp.concatenate(lhs, axis=1).astype(bf16)
            kt = k_buf[b, pl.ds(6 * i, 6)].reshape(2 * DH, W)
            s = jnp.dot(lhs, kt, preferred_element_type=f32) * (DH ** -0.5)
            e = jnp.exp(s - jnp.max(s, axis=-1, keepdims=True))
            p_buf[b, i] = e / jnp.sum(e, axis=-1, keepdims=True)
        return step

    def weighted_values(b):
        def step(i):
            for g in range(6):
                p = p_buf[b, i, pl.ds(g // 3, 1), :]
                o = jnp.sum(v_buf[b, 6 * i + g].astype(f32) * p, axis=-1, keepdims=True)
                o_col[b, pl.ds((6 * i + g) * 8, 8)] = jnp.broadcast_to(o, (64, 128)).reshape(8, 8, 128)
        return step

    def out_proj(b, j, gs, acc):
        a, r = _divmod(8 * j, 5)
        base = [a + _divmod(r + k, 5)[0] for k in range(5)]
        for g in gs:
            w = wo_buf[b, g, _rows(j, 64), :].astype(f32)
            for i in range(8):
                a2, k = divmod(256 * g + i, 5)
                acc[k] = acc[k] + w[8 * i:8 * i + 8] * o_col[b, base[k] + a2]
        return acc

    def out_sweeps(b, lo, n, num_groups=15):
        def body(j, carry):
            j = lo + j
            if b == 1:
                wait(wo_buf.at[1, pl.ds(0, num_groups), _rows(j, 64)], sweep_sems.at[j])
            slot = [_divmod(k + 3 * j, 5)[1] for k in range(5)]
            acc = out_proj(b, j, range(num_groups), [out_acc[b, s] for s in slot])
            for s, v in zip(slot, acc):
                out_acc[b, s] = v
            return carry
        lax.fori_loop(0, n, body, 0)

    def out_copy(b):
        half = (slice(None), slice(None), pl.ds(b * D, D))
        return pltpu.make_async_copy(out_buf.at[half], out_hbm.at[half], sems.at[8 + b])

    def write_out(b, acc):
        for c in range(5):
            out_buf[0, :, pl.ds(b * D + 128 * c, 128)] = jnp.sum(acc[c], axis=0, keepdims=True).astype(bf16)
        out_copy(b).start()

    bufs = [wq_buf.at[0], wq_buf.at[1], k_buf.at[0], k_buf.at[1], v_buf.at[0], v_buf.at[1], wo_buf.at[0]]
    streams = [
        wq_stream(awq, bufs[0], sems.at[0]), wq_stream(bwq, bufs[1], sems.at[1]),
        kv_stream(ak, bufs[2], sems.at[2]), kv_stream(bk, bufs[3], sems.at[3]),
        kv_stream(av, bufs[4], sems.at[4]), kv_stream(bv, bufs[5], sems.at[5]),
        wo_stream(awo, bufs[6], lambda j: sems.at[6]),
        wo_stream(bwo, wo_buf.at[1], lambda j: sweep_sems.at[j]),
    ]
    jobs = [(15, q_proj(0)), (15, q_proj(1)), (16, attention_probs(0)), (16, attention_probs(1)),
            (16, weighted_values(0)), (16, weighted_values(1)), (8, lambda i: out_sweeps(0, 4 * i, 4))]

    handover(None, streams[0])
    x_copies = [pltpu.make_async_copy(x, x_buf.at[b], sems.at[7]) for b, x in enumerate((ax, bx))]
    for c in x_copies:
        c.start()
    run(streams[0], 0, 14)
    q_acc[...] = jnp.zeros(q_acc.shape, f32)
    out_acc[...] = jnp.zeros(out_acc.shape, f32)
    for c in x_copies:
        c.wait()
    repeat_x()
    run(streams[0], 14, 28)

    for s, (steps, step) in enumerate(jobs):
        stream = streams[s + 1]
        end = 32 - LEAD // stream[0]
        start = 8 if s == 6 else end - steps
        handover(streams[s], stream)
        run(stream, 0, start)
        wait(bufs[s], sems.at[s])
        run(stream, start, start + steps, step)

    write_out(0, [out_acc[0, c] for c in range(5)])

    def held_back(i, u, prio):
        idx = (14, _rows(40 + u, 32))
        return pltpu.make_async_copy(bwo.at[idx], wo_buf.at[1].at[idx], sweep_sems.at[32 + u // 6])

    stream = wo_stream(bwo, wo_buf.at[1], lambda j: sweep_sems.at[j], num_groups=14)
    run(stream, 16, 18)
    run(stream, 18, 28, lambda i: out_sweeps(1, 2 * i, 2))
    handover(stream, (LEAD, held_back))
    out_sweeps(1, 20, 11, num_groups=14)
    acc = [out_acc[1, c] for c in range(5)]
    last = [(31, range(31, 32), range(14))]
    last += [(32 + n, range(20 + 3 * n, 23 + 3 * n), range(14, 15)) for n in range(4)]
    for sem, js, gs in last:
        wait(wo_buf.at[1, pl.ds(gs[0], len(gs)), pl.ds(64 * js[0], 64 * len(js))], sweep_sems.at[sem])
        for j in js:
            acc = out_proj(1, j, gs, [acc[(k + 3 * j) % 5] for k in range(5)])
            acc = [acc[(c - 3 * j) % 5] for c in range(5)]
    write_out(1, acc)
    out_copy(0).wait()
    out_copy(1).wait()


@jax.jit
def pallas_concat_heads__sliding_block_cached__sliding_block_cached__decode_kernel(
    A_x: jax.Array,
    A_k_cache: jax.Array,
    A_v_cache: jax.Array,
    A_wq: jax.Array,
    A_wo: jax.Array,
    B_x: jax.Array,
    B_k_cache: jax.Array,
    B_v_cache: jax.Array,
    B_wq: jax.Array,
    B_wo: jax.Array,
):
    def kv_view(t):
        return jnp.swapaxes(t, 2, 3).reshape(96, 64, SK)

    def wq_view(t):
        return t.reshape(80, 8, 6, 1024).transpose(0, 2, 1, 3).reshape(15, 256, 1024)

    def wo_view(t):
        return t.reshape(768, 8, 5, 128).transpose(0, 2, 1, 3).reshape(15, 2048, 128)

    hbm = pl.BlockSpec(memory_space=pltpu.HBM)
    return pl.pallas_call(
        _kernel,
        in_specs=[hbm] * 10,
        out_specs=hbm,
        out_shape=jax.ShapeDtypeStruct((1, 1, 2 * D), bf16),
        scratch_shapes=[
            pltpu.VMEM((2, 15, 256, 1024), bf16),
            pltpu.VMEM((2, 96, 64, W), bf16),
            pltpu.VMEM((2, 96, 64, W), bf16),
            pltpu.VMEM((2, 15, 2048, 128), bf16),
            pltpu.VMEM((2, 1, 1, D), bf16),
            pltpu.VMEM((6, 16, 128), f32),
            pltpu.VMEM((2, 8, 8, 128), f32),
            pltpu.VMEM((2, H // 2, 8, W), f32),
            pltpu.VMEM((2, 768, 8, 128), f32),
            pltpu.VMEM((2, 5, 8, 128), f32),
            pltpu.VMEM((1, 1, 2 * D), bf16),
            pltpu.SemaphoreType.DMA((10,)),
            pltpu.SemaphoreType.DMA((36,)),
        ],
        compiler_params=pltpu.CompilerParams(
            vmem_limit_bytes=100 * 2**20,
            disable_bounds_checks=True,
            disable_semaphore_checks=True,
        ),
    )(A_x, kv_view(A_k_cache), kv_view(A_v_cache), wq_view(A_wq), wo_view(A_wo),
      B_x, kv_view(B_k_cache), kv_view(B_v_cache), wq_view(B_wq), wo_view(B_wo))
```
